```python
import jax
import jax.numpy as jnp

def _softmax(x, axis=-1):
    return jax.nn.softmax(x, axis=axis)
def _gelu(x):
    return jax.nn.gelu(x, approximate=True)
def _silu(x):
    return jax.nn.silu(x)
def _sigmoid(x):
    return jax.nn.sigmoid(x)
def _layernorm(x, axis=-1, eps=1e-5):
    m = jnp.mean(x, axis=axis, keepdims=True)
    v = jnp.var(x, axis=axis, keepdims=True)
    return (x - m) / jnp.sqrt(v + eps)
def _scatter_add(tgt, idx, src, axis=0):
    return tgt.at[idx].add(src)
def _segment_sum(src, seg, n):
    return jax.ops.segment_sum(src, seg, n)
class _Rng:
    def __init__(self, key):
        self._k = key
    def _next(self):
        self._k, sub = jax.random.split(self._k)
        return sub
    def normal(self, shape):
        return jax.random.normal(self._next(), shape, dtype=jnp.bfloat16)
    def randint(self, lo, hi, shape):
        return jax.random.randint(self._next(), shape, lo, hi, dtype=jnp.int32)
    def uniform(self, shape, lo=0.0, hi=1.0):
        return jax.random.uniform(self._next(), shape, jnp.bfloat16, lo, hi)
    def permutation(self, n):
        return jax.random.permutation(self._next(), n)


kernel_name = 'concat_heads__spectral_gfnet__compressed_kv_cla__prompt'

def setup_inputs():
    _rng = _Rng(jax.random.key(int.from_bytes(__import__("os").urandom(4), "little")))
    _w = (lambda a: (lambda t: t.astype(jnp.bfloat16) if jnp.issubdtype(t.dtype, jnp.floating) else t)(jnp.asarray(a)))
    def _A_setup():
        B, S, D = 1, 2048, 448
        Df = D // 2 + 1
        return {
            "x": _w((lambda *s: _rng.normal(s) * 0.05)(B, S, D)),
            "w_r": _w((lambda *s: _rng.normal(s) * 0.05)(S, Df) * 0.02),
            "w_i": _w((lambda *s: _rng.normal(s) * 0.05)(S, Df) * 0.02),
        }
    _A_in = _A_setup()

    def _B_setup():
        B, H, Sq, Sk, D, M = 1, 16, 2048, 2048, 256, 448
        Dc = 4 * D
        return {
            "x": _w((lambda *s: _rng.normal(s) * 0.05)(B, Sq, M)),
            "c_kv": _w((lambda *s: _rng.normal(s) * 0.05)(B, Sk, Dc)),
            "w_q": _w((lambda *s: _rng.normal(s) * 0.05)(M, H, D) * (M ** -0.5)),
            "w_uk": _w((lambda *s: _rng.normal(s) * 0.05)(Dc, H, D) * (Dc ** -0.5)),
            "w_uv": _w((lambda *s: _rng.normal(s) * 0.05)(Dc, H, D) * (Dc ** -0.5)),
            "w_o": _w((lambda *s: _rng.normal(s) * 0.05)(H, D, M) * ((H * D) ** -0.5)),
        }
    _B_in = _B_setup()

    return {
        "A_x": _A_in["x"],
        "A_w_r": _A_in["w_r"],
        "A_w_i": _A_in["w_i"],
        "B_x": _B_in["x"],
        "B_c_kv": _B_in["c_kv"],
        "B_w_q": _B_in["w_q"],
        "B_w_uk": _B_in["w_uk"],
        "B_w_uv": _B_in["w_uv"],
        "B_w_o": _B_in["w_o"],
    }

def reference(A_x, A_w_r, A_w_i, B_x, B_c_kv, B_w_q, B_w_uk, B_w_uv, B_w_o):
    def _A_ref(x, w_r, w_i):
        B, S, D = x.shape
        X = (lambda x, axes=(-2,-1): jnp.fft.rfft2(x.astype(jnp.float32), axes=axes))(x, axes=(-2, -1))
        W = w_r + 1j * w_i
        X = X * W
        y = (lambda x, s, axes=(-2,-1): jnp.fft.irfft2(x, s=s, axes=axes).astype(jnp.bfloat16))(X, (S, D), axes=(-2, -1))
        return y

    def _B_ref(x, c_kv, w_q, w_uk, w_uv, w_o):
        B, Sq, M = x.shape[0], x.shape[1], x.shape[2]
        Sk = c_kv.shape[1]
        H, D = w_q.shape[1], w_q.shape[2]
        q = jnp.einsum("bqm,mhd->bhqd", x, w_q)
        k = jnp.einsum("bkc,chd->bhkd", c_kv, w_uk)
        v = jnp.einsum("bkc,chd->bhkd", c_kv, w_uv)
        scores = jnp.einsum("bhqd,bhkd->bhqk", q, k) * (D ** -0.5)
        off = Sk - Sq
        qi = jnp.arange(Sq)[:, None]
        kj = jnp.arange(Sk)[None, :]
        cmask = kj <= (qi + off)
        scores = jnp.where(cmask[None, None], scores, -1e9)
        p = _softmax(scores, axis=-1)
        ctx = jnp.einsum("bhqk,bhkd->bhqd", p, v)
        return jnp.einsum("bhqd,hdm->bqm", ctx, w_o)

    a = _A_ref(A_x, A_w_r, A_w_i)
    b = _B_ref(B_x, B_c_kv, B_w_q, B_w_uk, B_w_uv, B_w_o)
    return jnp.concatenate([a, b], axis=-1)
```

```python
import functools
import numpy as np
import jax
import jax.numpy as jnp
from jax import lax
import jax.experimental.pallas as pl
import jax.experimental.pallas.tpu as pltpu

S = 2048; DA = 448; DF = 225; H = 16; HD = 256; DC = 1024; M = 448
KP = 256
MP = 512
SH = MP - M


def _bf16(a):
    return np.asarray(a, dtype=np.float32).astype(jnp.bfloat16)


def _consts():
    d = np.arange(DA)[:, None].astype(np.float64)
    k = np.arange(DF)[None, :].astype(np.float64)
    ang = 2 * np.pi * ((d * k) % DA) / DA
    fd = np.zeros((DA, 2 * KP))
    fd[:, :DF] = np.cos(ang)
    fd[:, KP:KP + DF] = -np.sin(ang)
    fd[:, KP] = 0.0
    fd[:, KP + DF - 1] = 0.0
    wk = np.full((DF,), 2.0); wk[0] = 1.0; wk[-1] = 1.0
    fi = np.zeros((2 * KP, MP))
    fi[:DF, :DA] = (np.cos(ang) * wk[None, :]).T / (S * DA)
    si = -np.sin(ang); si[:, 0] = 0; si[:, -1] = 0
    fi[KP:KP + DF, :DA] = (si * wk[None, :]).T / (S * DA)
    m1 = np.zeros((16, 256, 128)); m1i = np.zeros((16, 256, 128))
    a16 = np.arange(16)
    for g in range(16):
        for c in range(8):
            s2 = 8 * g + c
            th = 2 * np.pi * (np.outer(a16, a16) % 16 / 16.0 + (a16[:, None] * s2) / S)
            rows = a16 * 8 + c
            m1[g][np.ix_(rows, rows)] = np.cos(th)
            m1[g][np.ix_(128 + rows, rows)] = -np.sin(th)
            m1i[g][np.ix_(rows, rows)] = np.cos(th.T)
            m1i[g][np.ix_(128 + rows, rows)] = np.sin(th.T)
    a128 = np.arange(128)
    th = 2 * np.pi * (np.outer(a128, a128) % 128) / 128.0
    m2 = np.concatenate([np.cos(th), -np.sin(th)], 0)
    m2i = np.concatenate([np.cos(th), np.sin(th)], 0)
    m2b = np.stack([m2, m2i], 0)
    p = np.zeros((128, 128))
    for f1 in range(16):
        for f2l in range(8):
            p[f1 * 8 + f2l, 16 * f2l + f1] = 1.0
    return _bf16(fd), _bf16(fi), _bf16(np.stack([m1, m1i], 0).reshape(32, 256, 128)), _bf16(m2b), _bf16(p)


_FD, _FI, _M1, _M2, _P = _consts()


def _cmul_stage(mat, data):
    o = jnp.dot(mat, data, preferred_element_type=jnp.float32)
    re = o[:128, :KP] - o[128:, KP:]
    im = o[:128, KP:] + o[128:, :KP]
    return re, im


TQ = 512
TK = 512
TD = 128
TP = 1024
UG = 4
NCH = 4
RCH = S // NCH
NT_DIMS = (((1,), (1,)), ((), ()))
TN_DIMS = (((0,), (0,)), ((), ()))
C_EXP = (HD ** -0.5) * 1.4426950408889634


def _rows_cat(parts):
    return parts[0] if len(parts) == 1 else jnp.concatenate(parts, axis=0)


def _ragged_reduce(pieces, op, nd):
    out = []
    for g in range(nd):
        acc = None
        for t in range(g + 1):
            x = pieces[t][(g - t) * TD:(g - t + 1) * TD]
            acc = x if acc is None else op(acc, x)
        out.append(acc)
    return _rows_cat(out)


def _kernel(fd_ref, m2_ref, p_ref,
            xa_hbm, wr_hbm, wi_hbm, xb_hbm, ckv_hbm, wq_hbm, wuk_hbm, wuv_hbm, wo_hbm, fi_hbm, m1_hbm,
            o_hbm,
            xa_ref, wr_ref, wi_ref, xb_ref, ckv_ref, fi_ref, m1_ref,
            wq_buf, wuk_buf, wuv_buf, wo_buf, wq_s, wuk_s, wuv_s,
            z_ref, t_ref, wp_ref, x_ref, q_ref, k_ref, v_ref, acc_ref, ost_ref,
            sem_xa, sem_in, sem_w, sem_wo, sem_out):
    wq32 = wq_hbm.bitcast(jnp.uint32)
    wuk32 = wuk_hbm.bitcast(jnp.uint32)
    wuv32 = wuv_hbm.bitcast(jnp.uint32)

    def xa_copy(i):
        c = pl.ds(pl.multiple_of(i * RCH, RCH), RCH)
        return pltpu.make_async_copy(xa_hbm.at[:, c], xa_ref.at[:, c], sem_xa.at[i])

    m1f_copy = pltpu.make_async_copy(m1_hbm.at[pl.ds(0, 16)], m1_ref.at[pl.ds(0, 16)], sem_in.at[0])
    wr_copy = pltpu.make_async_copy(wr_hbm, wr_ref, sem_in.at[1])
    wi_copy = pltpu.make_async_copy(wi_hbm, wi_ref, sem_in.at[2])
    m1i_copy = pltpu.make_async_copy(m1_hbm.at[pl.ds(16, 16)], m1_ref.at[pl.ds(16, 16)], sem_in.at[3])
    xb_copy = pltpu.make_async_copy(xb_hbm, xb_ref, sem_in.at[4])
    ckv_copy = pltpu.make_async_copy(ckv_hbm, ckv_ref, sem_in.at[5])
    fi_copy = pltpu.make_async_copy(fi_hbm, fi_ref, sem_in.at[6])

    def w_copies(j, slot):
        return (
            pltpu.make_async_copy(wq32.at[:, j, :], wq_buf.at[slot], sem_w.at[slot]),
            pltpu.make_async_copy(wuk32.at[:, j, :], wuk_buf.at[slot], sem_w.at[slot]),
            pltpu.make_async_copy(wuv32.at[:, j, :], wuv_buf.at[slot], sem_w.at[slot]),
        )

    def wo_copy(h, slot):
        return pltpu.make_async_copy(wo_hbm.at[h], wo_buf.at[slot, pl.ds(SH, M), :], sem_wo.at[slot])

    def out_copy(i):
        r = pl.ds(pl.multiple_of(i * RCH, RCH), RCH)
        return pltpu.make_async_copy(ost_ref.at[r, :], o_hbm.at[r, :], sem_out.at[i])

    for i in range(NCH):
        xa_copy(i).start()
    m1f_copy.start()
    wr_copy.start()
    wi_copy.start()

    wo_buf[:, 0:SH, :] = jnp.zeros((2, SH, HD), jnp.bfloat16)

    def fwd_d(i, _):
        c = pl.ds(pl.multiple_of(i * RCH, RCH), RCH)
        xa_copy(i).wait()
        z = lax.dot_general(xa_ref[:, c], fd_ref[...], TN_DIMS, preferred_element_type=jnp.float32)
        z_ref[pl.ds(i * (RCH // 128), RCH // 128)] = z.reshape(RCH // 128, 128, 2 * KP)
        acc_ref[c, :] = jnp.zeros((RCH, MP), jnp.float32)
    lax.fori_loop(0, NCH, fwd_d, None)

    m1i_copy.start()
    xb_copy.start()
    ckv_copy.start()
    for cp in w_copies(0, 0):
        cp.start()
    wo_copy(0, 0).start()
    fi_copy.start()

    def stage1(base, src, dst, extra=None):
        def body(g4, _):
            for u in range(UG):
                g = g4 * UG + u
                r8 = pl.ds(pl.multiple_of(g * 8, 8), 8)
                d = src[:, r8, :].reshape(128, 2 * KP).astype(jnp.bfloat16)
                re, im = _cmul_stage(m1_ref[base + g], d)
                dst[:, r8, :KP] = re.reshape(16, 8, KP)
                dst[:, r8, KP:] = im.reshape(16, 8, KP)
            if extra is not None:
                extra(g4)
        lax.fori_loop(0, 16 // UG, body, None)

    m1f_copy.wait()
    stage1(0, z_ref, t_ref)

    wr_copy.wait()
    wi_copy.wait()

    def perm_w(a2, _):
        for u in range(4):
            a = a2 * 4 + u
            c = pl.ds(pl.multiple_of(a * 128, 128), 128)
            r8 = pl.ds(pl.multiple_of(a * 8, 8), 8)
            for j, w_ref in enumerate((wr_ref, wi_ref)):
                wp = lax.dot_general(p_ref[...], w_ref[:, c], NT_DIMS, preferred_element_type=jnp.float32)
                wp = jnp.concatenate([wp, jnp.zeros((128, KP - DF), jnp.float32)], axis=1)
                wp_ref[:, r8, j * KP:(j + 1) * KP] = wp.reshape(16, 8, KP)
    lax.fori_loop(0, 4, perm_w, None)

    def mid(f4, _):
        for u in range(4):
            f1 = f4 * 4 + u
            d = t_ref[f1].astype(jnp.bfloat16)
            xr, xi = _cmul_stage(m2_ref[0], d)
            wr = wp_ref[f1, :, :KP]; wi = wp_ref[f1, :, KP:]
            yr = xr * wr - xi * wi
            yi = xr * wi + xi * wr
            d2 = jnp.concatenate([yr, yi], axis=1).astype(jnp.bfloat16)
            ur, ui = _cmul_stage(m2_ref[1], d2)
            z_ref[f1, :, :KP] = ur
            z_ref[f1, :, KP:] = ui
    lax.fori_loop(0, 4, mid, None)

    m1i_copy.wait()
    xb_copy.wait()

    def xb_transpose(g4):
        c = pl.ds(pl.multiple_of(g4 * (S // (16 // UG)), S // (16 // UG)), S // (16 // UG))
        x_ref[c, :] = xb_ref[:, c].T
    stage1(16, z_ref, t_ref, xb_transpose)

    ckv_copy.wait()

    def head(h, _):
        j = h // 2
        hh = h % 2
        slot = j % 2
        oslot = h % 2

        @pl.when(hh == 0)
        def _():
            for cp in w_copies(j, slot):
                cp.wait()

            @pl.when(j + 1 < H // 2)
            def _():
                for cp in w_copies(j + 1, 1 - slot):
                    cp.start()

        wo_copy(h, oslot).wait()

        @pl.when(h + 1 < H)
        def _():
            wo_copy(h + 1, 1 - oslot).start()

        sh = (16 - 16 * hh).astype(jnp.uint32)

        def unpack(buf):
            x = (buf[slot] << sh) & jnp.uint32(0xFFFF0000)
            return pltpu.bitcast(x, jnp.float32).astype(jnp.bfloat16)

        wq_s[...] = unpack(wq_buf)
        wuk_s[...] = unpack(wuk_buf)
        wuv_s[...] = unpack(wuv_buf)

        def proj(i, _):
            r = pl.ds(pl.multiple_of(i * TP, TP), TP)
            q_ref[r, :] = jnp.dot(x_ref[r, :], wq_s[...], preferred_element_type=jnp.float32).astype(jnp.bfloat16)
            c = ckv_ref[r, :]
            k_ref[r, :] = jnp.dot(c, wuk_s[...], preferred_element_type=jnp.float32).astype(jnp.bfloat16)
            v_ref[r, :] = jnp.dot(c, wuv_s[...], preferred_element_type=jnp.float32).astype(jnp.bfloat16)
        lax.fori_loop(0, S // TP, proj, None)

        nd = TQ // TD
        tri = lax.broadcasted_iota(jnp.int32, (TD, TD), 1) <= lax.broadcasted_iota(jnp.int32, (TD, TD), 0)
        for i in range(S // TQ):
            R0 = i * TQ
            q = q_ref[R0:R0 + TQ, :]
            sp = []
            for t in range(nd):
                kk = k_ref[R0 + t * TD:R0 + (t + 1) * TD, :]
                s = lax.dot_general(q[t * TD:], kk, NT_DIMS, preferred_element_type=jnp.float32)
                s0 = jnp.where(tri, s[:TD], -1e30)
                s = _rows_cat([s0, s[TD:]]) if t < nd - 1 else s0
                sp.append(s)
            m = jnp.max(_ragged_reduce(sp, jnp.maximum, nd), axis=1, keepdims=True)
            pp = [jnp.exp2((sp[t] - m[t * TD:]) * C_EXP) for t in range(nd)]
            lp = _ragged_reduce(pp, jnp.add, nd)
            pv = []
            for t in range(nd):
                vv = v_ref[R0 + t * TD:R0 + (t + 1) * TD, :]
                pv.append(jnp.dot(pp[t].astype(jnp.bfloat16), vv, preferred_element_type=jnp.float32))
            acc = _ragged_reduce(pv, jnp.add, nd)
            for jj in range(i):
                kk = k_ref[jj * TK:(jj + 1) * TK, :]
                vv = v_ref[jj * TK:(jj + 1) * TK, :]
                s = lax.dot_general(q, kk, NT_DIMS, preferred_element_type=jnp.float32)
                m_new = jnp.maximum(m, jnp.max(s, axis=1, keepdims=True))
                alpha = jnp.exp2((m - m_new) * C_EXP)
                p = jnp.exp2((s - m_new) * C_EXP)
                ps = p[:, 0:TD]
                for u in range(1, TK // TD):
                    ps = ps + p[:, u * TD:(u + 1) * TD]
                lp = alpha * lp + ps
                acc = alpha * acc + jnp.dot(p.astype(jnp.bfloat16), vv, preferred_element_type=jnp.float32)
                m = m_new
            l = jnp.sum(lp, axis=1, keepdims=True)
            ctx = (acc * (1.0 / l)).astype(jnp.bfloat16)
            po = lax.dot_general(ctx, wo_buf[oslot], NT_DIMS, preferred_element_type=jnp.float32)
            acc_ref[R0:R0 + TQ, :] += po
    lax.fori_loop(0, H, head, None)

    fi_copy.wait()

    def inv_d(i, _):
        r = pl.ds(pl.multiple_of(i * RCH, RCH), RCH)
        d = t_ref[pl.ds(i * (RCH // 128), RCH // 128)].reshape(RCH, 2 * KP).astype(jnp.bfloat16)
        y = jnp.dot(d, fi_ref[...], preferred_element_type=jnp.float32)
        b = acc_ref[r, :]
        ost_ref[r, 0:384] = y[:, 0:384].astype(jnp.bfloat16)
        ost_ref[r, 384:512] = (y[:, 384:512] + b[:, 0:128]).astype(jnp.bfloat16)
        ost_ref[r, 512:896] = b[:, 128:512].astype(jnp.bfloat16)
        out_copy(i).start()
    lax.fori_loop(0, NCH, inv_d, None)
    for i in range(NCH):
        out_copy(i).wait()


@jax.jit
def pallas_concat_heads__spectral_gfnet__compressed_kv_cla__prompt_kernel(
    A_x, A_w_r, A_w_i, B_x, B_c_kv, B_w_q, B_w_uk, B_w_uv, B_w_o):
    xa = A_x.reshape(S, DA).T
    xb = B_x.reshape(S, M).T
    ckv = B_c_kv.reshape(S, DC)
    wo = jnp.transpose(B_w_o, (0, 2, 1))
    vmem = pl.BlockSpec(memory_space=pltpu.VMEM)
    hbm = pl.BlockSpec(memory_space=pl.ANY)
    bf = jnp.bfloat16
    out = pl.pallas_call(
        _kernel,
        in_specs=[vmem] * 3 + [hbm] * 11,
        out_specs=hbm,
        out_shape=jax.ShapeDtypeStruct((S, 2 * DA), bf),
        scratch_shapes=[
            pltpu.VMEM((DA, S), bf), pltpu.VMEM((DF, S), bf), pltpu.VMEM((DF, S), bf),
            pltpu.VMEM((M, S), bf), pltpu.VMEM((S, DC), bf), pltpu.VMEM((2 * KP, MP), bf),
            pltpu.VMEM((32, 256, 128), bf),
            pltpu.VMEM((2, M, HD), jnp.uint32), pltpu.VMEM((2, DC, HD), jnp.uint32),
            pltpu.VMEM((2, DC, HD), jnp.uint32), pltpu.VMEM((2, MP, HD), bf),
            pltpu.VMEM((M, HD), bf), pltpu.VMEM((DC, HD), bf), pltpu.VMEM((DC, HD), bf),
            pltpu.VMEM((16, 128, 2 * KP), jnp.float32),
            pltpu.VMEM((16, 128, 2 * KP), jnp.float32),
            pltpu.VMEM((16, 128, 2 * KP), jnp.float32),
            pltpu.VMEM((S, M), bf),
            pltpu.VMEM((S, HD), bf), pltpu.VMEM((S, HD), bf), pltpu.VMEM((S, HD), bf),
            pltpu.VMEM((S, MP), jnp.float32),
            pltpu.VMEM((S, 2 * DA), bf),
            pltpu.SemaphoreType.DMA((NCH,)), pltpu.SemaphoreType.DMA((7,)),
            pltpu.SemaphoreType.DMA((2,)), pltpu.SemaphoreType.DMA((2,)),
            pltpu.SemaphoreType.DMA((NCH,)),
        ],
        compiler_params=pltpu.CompilerParams(vmem_limit_bytes=100 * 1024 * 1024),
    )(_FD, _M2, _P, xa, A_w_r.T, A_w_i.T, xb, ckv, B_w_q, B_w_uk, B_w_uv, wo, _FI, _M1)
    return out.reshape(1, S, 2 * DA)
```

```python
import numpy as np
import jax
import jax.numpy as jnp
from jax import lax
import jax.experimental.pallas as pl
import jax.experimental.pallas.tpu as pltpu

S = 2048
DA = 448
DF = DA // 2 + 1
H = 16
HD = 256
DC = 1024
M = 448
KP = 256
MP = 512
SH = MP - M

TQ = 512
TD = 128
UG = 8
UM = 8
NCH = 4
RCH = S // NCH
NOUT = 8
ROUT = S // NOUT

NT_DIMS = (((1,), (1,)), ((), ()))
C_EXP = (HD ** -0.5) * 1.4426950408889634
NEG = -1e30

ORDER = "K0 K1 K2 Q2 q2 s2 K3 V0 V1 Q3 q3 s3 V2 V3 p2 Q1 q1 s1 p3 Q0 q0 s0 o2 p1 o3 p0 o1 o0".split()


def _bf16(a):
    return np.asarray(a, dtype=np.float32).astype(jnp.bfloat16)


def _consts():
    d = np.arange(DA, dtype=np.int64)[:, None]
    k = np.arange(DF, dtype=np.int64)[None, :]
    ang = 2 * np.pi * ((d * k) % DA) / DA
    si = -np.sin(ang)
    si[:, 0] = 0.0
    si[:, -1] = 0.0
    fd = np.zeros((DA, 2 * KP))
    fd[:, :DF] = np.cos(ang)
    fd[:, KP:KP + DF] = si
    wk = np.full((DF,), 2.0)
    wk[0] = wk[-1] = 1.0
    fi = np.zeros((2 * KP, MP))
    fi[:DF, :DA] = (np.cos(ang) * wk[None, :]).T / (S * DA)
    fi[KP:KP + DF, :DA] = (si * wk[None, :]).T / (S * DA)
    m1 = np.zeros((2, 16, 256, 128))
    a16 = np.arange(16, dtype=np.int64)
    for g in range(16):
        for c in range(8):
            s2 = 8 * g + c
            th = 2 * np.pi * ((np.outer(a16, a16) * 128 + a16[:, None] * s2) % S) / S
            rows = a16 * 8 + c
            m1[0, g][np.ix_(rows, rows)] = np.cos(th)
            m1[0, g][np.ix_(128 + rows, rows)] = -np.sin(th)
            m1[1, g][np.ix_(rows, rows)] = np.cos(th.T)
            m1[1, g][np.ix_(128 + rows, rows)] = np.sin(th.T)
    a128 = np.arange(128, dtype=np.int64)
    th = 2 * np.pi * (np.outer(a128, a128) % 128) / 128
    m2 = np.stack([np.concatenate([np.cos(th), -np.sin(th)], 0),
                   np.concatenate([np.cos(th), np.sin(th)], 0)], 0)
    perm = np.zeros((128, 128))
    for f1 in range(16):
        for f2l in range(8):
            perm[f1 * 8 + f2l, 16 * f2l + f1] = 1.0
    return _bf16(fd), _bf16(fi), _bf16(m1.reshape(32, 256, 128)), _bf16(m2), _bf16(perm)


_FD, _FI, _M1, _M2, _PERM = _consts()


def _cmatmul(mat, data):
    o = jnp.dot(mat, data, preferred_element_type=jnp.float32)
    return o[:128, :KP] - o[128:, KP:], o[:128, KP:] + o[128:, :KP]


def _cat(parts, axis):
    return parts[0] if len(parts) == 1 else jnp.concatenate(parts, axis=axis)


def _half(start, size):
    if isinstance(start, int):
        return slice(start // 2, (start + size) // 2)
    return pl.ds(pl.multiple_of(start // 2, size // 2), size // 2)


def _ld(ref3, start, size):
    rows = _half(start, size)
    return _cat([pltpu.bitcast(ref3[t, rows, :], jnp.bfloat16) for t in range(ref3.shape[0])], 1)


def _st(ref3, start, val):
    rows = _half(start, val.shape[0])
    v = val.astype(jnp.bfloat16)
    for t in range(ref3.shape[0]):
        ref3[t, rows, :] = pltpu.bitcast(v[:, t * 128:(t + 1) * 128], jnp.uint32)


def _ragged_sum(pieces):
    out = []
    for g in range(TQ // TD):
        acc = None
        for t in range(g + 1):
            x = pieces[t][(g - t) * TD:(g - t + 1) * TD]
            acc = x if acc is None else acc + x
        out.append(acc)
    return _cat(out, 0)


def _kernel(xa_hbm, wr_hbm, wi_hbm, xb_hbm, ckv_hbm, wq_hbm, wuk_hbm, wuv_hbm, wo_hbm,
            fd_hbm, fi_hbm, m1_hbm, m2_hbm, perm_hbm,
            o_hbm,
            xa_ref, xat_ref, wr_ref, wi_ref, xb_ref, fd_ref, fi_ref, m1_ref, m2_ref, perm_ref,
            z_ref, t_ref, wp_ref,
            ckv_ref, x_ref, wq_ref, wuk_ref, wuv_ref, wo_ref, q_ref, k_ref, v_ref,
            acc_ref, ost_ref,
            s0, s1, s2, s3, p0, p1, p2, p3, c0, c1, c2, c3,
            sem_xa, sem, sem_out):
    s_refs, p_refs, ctx_refs = (s0, s1, s2, s3), (p0, p1, p2, p3), (c0, c1, c2, c3)
    bf = jnp.bfloat16
    copy = pltpu.make_async_copy
    wq32, wuk32, wuv32 = (r.bitcast(jnp.uint32) for r in (wq_hbm, wuk_hbm, wuv_hbm))
    ckv16, wo16 = ckv_ref.bitcast(bf), wo_ref.bitcast(bf)

    def xa_copy(i):
        c = pl.ds(pl.multiple_of(i * RCH, RCH), RCH)
        return copy(xa_hbm.at[:, c], xa_ref.at[:, c], sem_xa.at[i])

    def pair_copies(j, s):
        return [copy(wq32.at[:, j, :], wq_ref.at[j, pl.ds(0, M), :], s),
                copy(wuk32.at[:, j, :], wuk_ref.at[j], s),
                copy(wuv32.at[:, j, :], wuv_ref.at[j], s)]

    def wo_copies(h0, n, s):
        return [copy(wo_hbm.at[pl.ds(h0, n), :, pl.ds(t * 128, 128)], wo16.at[t, pl.ds(h0, n)], s)
                for t in range(HD // 128)]

    def out_copy(i):
        r = pl.ds(pl.multiple_of(i * ROUT, ROUT), ROUT)
        return copy(ost_ref.at[r, :], o_hbm.at[r, :], sem_out.at[i])

    g_fd = [copy(fd_hbm, fd_ref, sem.at[0])]
    g_st1 = [copy(perm_hbm, perm_ref, sem.at[1]), copy(m1_hbm.at[pl.ds(0, 16)], m1_ref.at[pl.ds(0, 16)], sem.at[1]),
             copy(wr_hbm, wr_ref, sem.at[1]), copy(wi_hbm, wi_ref, sem.at[1]), copy(m2_hbm, m2_ref, sem.at[1])]
    g_st1i = [copy(m1_hbm.at[pl.ds(16, 16)], m1_ref.at[pl.ds(16, 16)], sem.at[2]), copy(xb_hbm, xb_ref, sem.at[2])]
    g_h0 = ([copy(ckv_hbm.at[:, pl.ds(t * 128, 128)], ckv16.at[t], sem.at[3]) for t in range(DC // 128)]
            + pair_copies(0, sem.at[3]) + wo_copies(0, 2, sem.at[3]))
    g_rest = wo_copies(2, H - 2, sem.at[4]) + [c for j in range(1, H // 2) for c in pair_copies(j, sem.at[4])]
    g_fin = [copy(fi_hbm, fi_ref, sem.at[5])]

    w_h0 = [copy(ckv_ref, ckv_ref, sem.at[3])] + pair_copies(0, sem.at[3]) + [
        copy(wo_ref.at[:, pl.ds(0, 2)], wo_ref.at[:, pl.ds(0, 2)], sem.at[3])]
    rest = pl.ds(1, H // 2 - 1)
    w_rest = [copy(wq_ref.at[rest, pl.ds(0, M), :], wq_ref.at[rest, pl.ds(0, M), :], sem.at[4]),
              copy(wuk_ref.at[rest], wuk_ref.at[rest], sem.at[4]),
              copy(wuv_ref.at[rest], wuv_ref.at[rest], sem.at[4]),
              copy(wo_ref.at[:, pl.ds(2, H - 2)], wo_ref.at[:, pl.ds(2, H - 2)], sem.at[4])]

    def start(group):
        for c in group:
            c.start()

    def wait(group):
        for c in group:
            c.wait()

    xa_copy(0).start()
    start(g_fd)
    xa_copy(1).start()
    wq_ref[:, M:MP, :] = jnp.zeros((H // 2, MP - M, HD), jnp.uint32)

    def xa_transpose(i):
        c = pl.ds(pl.multiple_of(i * RCH, RCH), RCH)
        xat_ref[c, :] = xa_ref[:, c].T

    xa_copy(0).wait()
    for i in range(2, NCH):
        xa_copy(i).start()
    xa_transpose(0)
    wait(g_fd)

    def fwd_d(i, _):
        @pl.when(i + 1 < NCH)
        def _():
            xa_copy(i + 1).wait()

        @pl.when(i == 0)
        def _():
            start(g_st1)

        @pl.when(i == 2)
        def _():
            start(g_st1i)
            start(g_h0)

        c = pl.ds(pl.multiple_of(i * RCH, RCH), RCH)
        z = jnp.dot(xat_ref[c, :], fd_ref[...], preferred_element_type=jnp.float32)
        z_ref[pl.ds(i * (RCH // 128), RCH // 128)] = z.reshape(RCH // 128, 128, 2 * KP)
        xa_transpose(jnp.minimum(i + 1, NCH - 1))
    lax.fori_loop(0, NCH, fwd_d, None)

    def step16(base, extra):
        def body(g4, _):
            for u in range(UG):
                g = g4 * UG + u
                r8 = pl.ds(pl.multiple_of(g * 8, 8), 8)
                d = z_ref[:, r8, :].reshape(128, 2 * KP).astype(bf)
                re, im = _cmatmul(m1_ref[base + g], d)
                t_ref[:, r8, :KP] = re.reshape(16, 8, KP)
                t_ref[:, r8, KP:] = im.reshape(16, 8, KP)
            extra(g4)
        lax.fori_loop(0, 16 // UG, body, None)

    def perm_w(a4):
        for u in range(UG):
            a = a4 * UG + u
            c = pl.ds(pl.multiple_of(a * 128, 128), 128)
            r8 = pl.ds(pl.multiple_of(a * 8, 8), 8)
            for j, w_ref in enumerate((wr_ref, wi_ref)):
                wp = lax.dot_general(perm_ref[...], w_ref[:, c], NT_DIMS, preferred_element_type=jnp.float32)
                wp = jnp.concatenate([wp, jnp.zeros((128, KP - DF), jnp.float32)], axis=1)
                wp_ref[:, r8, j * KP:(j + 1) * KP] = wp.reshape(16, 8, KP)

    wait(g_st1)
    step16(0, perm_w)

    def step128(f4, _):
        def fwd(f1):
            return _cmatmul(m2_ref[0], t_ref[f1].astype(bf))

        def inv(f1, x):
            xr, xi = x
            wr = wp_ref[f1, :, :KP]
            wi = wp_ref[f1, :, KP:]
            y = jnp.concatenate([xr * wr - xi * wi, xr * wi + xi * wr], axis=1).astype(bf)
            ur, ui = _cmatmul(m2_ref[1], y)
            z_ref[f1, :, :KP] = ur
            z_ref[f1, :, KP:] = ui

        nz = S // (16 // UM)
        acc_ref[:, pl.ds(pl.multiple_of(f4 * nz, nz), nz)] = jnp.zeros((MP, nz), jnp.float32)
        x = fwd(f4 * UM)
        for u in range(UM):
            xn = fwd(f4 * UM + u + 1) if u + 1 < UM else None
            inv(f4 * UM + u, x)
            x = xn
    lax.fori_loop(0, 16 // UM, step128, None)

    def xb_transpose(g4):
        n = S // (16 // UG)
        c = pl.ds(pl.multiple_of(g4 * n, n), n)
        rows = _half(g4 * n, n)
        for t in range(M // 128):
            x_ref[t, rows, :] = pltpu.bitcast(xb_ref[t * 128:(t + 1) * 128, c].T, jnp.uint32)
        tail = jnp.concatenate([xb_ref[M - SH:M, c], jnp.zeros((SH, n), bf)], axis=0)
        x_ref[M // 128, rows, :] = pltpu.bitcast(tail.T, jnp.uint32)

    wait(g_st1i)
    step16(16, xb_transpose)

    wait(w_h0)
    start(g_rest)
    start(g_fin)
    nd = TQ // TD

    def head(h, _):
        @pl.when(h == 2)
        def _():
            wait(w_rest)

        j = h // 2
        lo = (16 - 16 * (h % 2)).astype(jnp.uint32)

        def unpack(buf):
            return pltpu.bitcast((buf[j] << lo) & jnp.uint32(0xFFFF0000), jnp.float32).astype(bf)

        def proj_q(i):
            q = jnp.dot(_ld(x_ref, i * TQ, TQ), unpack(wq_ref), preferred_element_type=jnp.float32)
            _st(q_ref, i * TQ, q * C_EXP)

        def proj_k(i):
            _st(k_ref, i * TQ, jnp.dot(_ld(ckv_ref, i * TQ, TQ), unpack(wuk_ref), preferred_element_type=jnp.float32))

        def proj_v(i):
            _st(v_ref, i * TQ, jnp.dot(_ld(ckv_ref, i * TQ, TQ), unpack(wuv_ref), preferred_element_type=jnp.float32))

        tri = lax.broadcasted_iota(jnp.int32, (TD, TD), 1) <= lax.broadcasted_iota(jnp.int32, (TD, TD), 0)
        lsum = {}

        def scores(i):
            r0 = i * TQ
            q = _ld(q_ref, r0, TQ)
            if i > 0:
                s_refs[i][:, 0:r0] = lax.dot_general(q, _ld(k_ref, 0, r0), NT_DIMS, preferred_element_type=jnp.float32)
            for t in range(nd):
                c = r0 + t * TD
                s = lax.dot_general(q[t * TD:], _ld(k_ref, c, TD), NT_DIMS, preferred_element_type=jnp.float32)
                s_refs[i][t * TD:(t + 1) * TD, c:c + TD] = jnp.where(tri, s[:TD], NEG)
                if t < nd - 1:
                    s_refs[i][(t + 1) * TD:, c:c + TD] = s[TD:]

        def softmax(i):
            ls = []
            for g in range(nd):
                w = i * TQ + (g + 1) * TD
                s = s_refs[i][g * TD:(g + 1) * TD, 0:w]
                p = jnp.exp2(s - jnp.max(s, axis=1, keepdims=True))
                ls.append(jnp.sum(p, axis=1, keepdims=True))
                p_refs[i][g * TD:(g + 1) * TD, 0:w] = p.astype(bf)
            lsum[i] = _cat(ls, 0)

        def pv(i):
            r0 = i * TQ
            acc = _ragged_sum([
                jnp.dot(p_refs[i][t * TD:, r0 + t * TD:r0 + (t + 1) * TD], _ld(v_ref, r0 + t * TD, TD),
                        preferred_element_type=jnp.float32) for t in range(nd)])
            if i > 0:
                acc = acc + jnp.dot(p_refs[i][:, 0:r0], _ld(v_ref, 0, r0), preferred_element_type=jnp.float32)
            ctx_refs[i][...] = (acc * (1.0 / lsum[i])).astype(bf)

        def oproj(i):
            wo_t = _cat([pltpu.bitcast(wo_ref[t, h], bf) for t in range(HD // 128)], 1)
            acc_ref[SH:, i * TQ:(i + 1) * TQ] += lax.dot_general(
                wo_t, ctx_refs[i][...], NT_DIMS, preferred_element_type=jnp.float32)

        ops = {"q": scores, "s": softmax, "p": pv, "o": oproj, "Q": proj_q, "K": proj_k, "V": proj_v}
        for op in ORDER:
            ops[op[0]](int(op[1]))
    lax.fori_loop(0, H, head, None)

    wait(g_fin)

    def inv_d(i2, _):
        for u in range(NOUT // NCH):
            i = i2 * (NOUT // NCH) + u
            r = pl.ds(pl.multiple_of(i * ROUT, ROUT), ROUT)
            d = t_ref[pl.ds(i * (ROUT // 128), ROUT // 128)].reshape(ROUT, 2 * KP).astype(bf)
            y = jnp.dot(d, fi_ref[...], preferred_element_type=jnp.float32)
            b = acc_ref[:, r].astype(bf).T
            ost_ref[r, 0:384] = y[:, 0:384].astype(bf)
            ost_ref[r, 384:512] = (y[:, 384:512] + b[:, 0:128].astype(jnp.float32)).astype(bf)
            ost_ref[r, 512:896] = b[:, 128:512]
            out_copy(i).start()
    lax.fori_loop(0, NCH, inv_d, None)
    for i in range(NOUT):
        out_copy(i).wait()


@jax.jit
def pallas_concat_heads__spectral_gfnet__compressed_kv_cla__prompt_kernel(
        A_x, A_w_r, A_w_i, B_x, B_c_kv, B_w_q, B_w_uk, B_w_uv, B_w_o):
    bf, u32, f32 = jnp.bfloat16, jnp.uint32, jnp.float32
    hbm = pl.BlockSpec(memory_space=pl.ANY)
    vm = pltpu.VMEM
    out = pl.pallas_call(
        _kernel,
        in_specs=[hbm] * 14,
        out_specs=hbm,
        out_shape=jax.ShapeDtypeStruct((S, DA + M), bf),
        scratch_shapes=[
            vm((DA, S), bf), vm((S, DA), bf), vm((DF, S), bf), vm((DF, S), bf), vm((M, S), bf),
            vm((DA, 2 * KP), bf), vm((2 * KP, MP), bf), vm((32, 256, 128), bf), vm((2, 256, 128), bf), vm((128, 128), bf),
            vm((16, 128, 2 * KP), f32), vm((16, 128, 2 * KP), f32), vm((16, 128, 2 * KP), f32),
            vm((DC // 128, S // 2, 128), u32), vm((MP // 128, S // 2, 128), u32),
            vm((H // 2, MP, HD), u32), vm((H // 2, DC, HD), u32), vm((H // 2, DC, HD), u32),
            vm((HD // 128, H, M // 2, 128), u32),
            vm((HD // 128, S // 2, 128), u32), vm((HD // 128, S // 2, 128), u32), vm((HD // 128, S // 2, 128), u32),
            vm((MP, S), f32), vm((S, DA + M), bf),
            *[vm((TQ, (i + 1) * TQ), f32) for i in range(S // TQ)],
            *[vm((TQ, (i + 1) * TQ), bf) for i in range(S // TQ)],
            *[vm((TQ, HD), bf) for i in range(S // TQ)],
            pltpu.SemaphoreType.DMA((NCH,)), pltpu.SemaphoreType.DMA((6,)), pltpu.SemaphoreType.DMA((NOUT,)),
        ],
        compiler_params=pltpu.CompilerParams(vmem_limit_bytes=110 * 1024 * 1024),
    )(A_x.reshape(S, DA).T, A_w_r.T, A_w_i.T, B_x.reshape(S, M).T, B_c_kv.reshape(S, DC),
      B_w_q, B_w_uk, B_w_uv, jnp.transpose(B_w_o, (0, 2, 1)), _FD, _FI, _M1, _M2, _PERM)
    return out.reshape(1, S, DA + M)
```
